```python
import os as _os
_os.environ.setdefault("JAX_PLATFORMS", "cpu")
import jax
import jax.numpy as jnp

def _softmax(x, axis=-1):
    return jax.nn.softmax(x, axis=axis)
def _gelu(x):
    return jax.nn.gelu(x, approximate=True)
def _silu(x):
    return jax.nn.silu(x)
def _sigmoid(x):
    return jax.nn.sigmoid(x)
def _layernorm(x, axis=-1, eps=1e-5):
    m = jnp.mean(x, axis=axis, keepdims=True)
    v = jnp.var(x, axis=axis, keepdims=True)
    return (x - m) / jnp.sqrt(v + eps)
def _scatter_add(tgt, idx, src, axis=0):
    return tgt.at[idx].add(src)
def _segment_sum(src, seg, n):
    return jax.ops.segment_sum(src, seg, n)
class _Rng:
    def __init__(self, key):
        self._k = key
    def _next(self):
        self._k, sub = jax.random.split(self._k)
        return sub
    def normal(self, shape):
        return jax.random.normal(self._next(), shape, dtype=jnp.bfloat16)
    def randint(self, lo, hi, shape):
        return jax.random.randint(self._next(), shape, lo, hi, dtype=jnp.int32)
    def uniform(self, shape, lo=0.0, hi=1.0):
        return jax.random.uniform(self._next(), shape, jnp.bfloat16, lo, hi)
    def permutation(self, n):
        return jax.random.permutation(self._next(), n)


kernel_name = 'standalone__sliding_local_fixed_window__prompt'

def setup_inputs():
    _rng = _Rng(jax.random.key(int.from_bytes(__import__("os").urandom(4), "little")))
    _w = (lambda a: (lambda t: t.astype(jnp.bfloat16) if jnp.issubdtype(t.dtype, jnp.floating) else t)(jnp.asarray(a)))
    B, H, S, D = 1, 32, 2048, 128
    return {
        "q": _w((lambda *s: _rng.normal(s) * 0.4)(B, H, S, D)),
        "k": _w((lambda *s: _rng.normal(s) * 0.4)(B, H, S, D)),
        "v": _w((lambda *s: _rng.normal(s) * 0.05)(B, H, S, D)),
    }

def reference(q, k, v):
    B, H, S, D = q.shape
    w = 32
    pos = jnp.arange(S)
    rel = pos[:, None] - pos[None, :]
    mask = (rel >= 0) & (rel < w)
    scores = jnp.einsum("bhqd,bhkd->bhqk", q, k) * (D ** -0.5)
    scores = jnp.where(mask[None, None], scores, (lambda x, dt: x.astype(dt))(jnp.array(-1e9), q.dtype))
    p = _softmax(scores, axis=-1)
    return jnp.einsum("bhqk,bhkd->bhqd", p, v)
```

```python
import math

import jax
import jax.numpy as jnp
from jax import lax
from jax.experimental import pallas as pl
from jax.experimental.pallas import tpu as pltpu

_W = 32
_TQ = 64
_TK = 128
_PAD = _TK - _TQ
_RR = 128
_L = 3
_WG = 16
_WNH = 8
_WR = 128


@jax.jit
def pallas_standalone__sliding_local_fixed_window__prompt_kernel(
    q: jax.Array,
    k: jax.Array,
    v: jax.Array,
):
    B, H, S, D = q.shape
    N = B * H * S
    GR = S
    NG = N // GR
    L = _L
    WS = N // _WG
    nwc = WS // _WR
    NWD = (_WG // _WNH) * nwc
    assert D == 128 and S % _RR == 0 and S % _TQ == 0 and NG > L
    assert N % _WG == 0 and WS % _WR == 0 and WS % S == 0
    c = (D ** -0.5) * math.log2(math.e)

    def w_last_row(j):
        g, cc = divmod(j, nwc)
        return (g * _WNH + _WNH - 1) * WS + (cc + 1) * _WR

    per_slot = max(1, (3 * GR) // (_WNH * _WR))
    sched, nxt = [], 0
    for g in range(NG - L, NG):
        lst = []
        while nxt < NWD and len(lst) < per_slot and w_last_row(nxt) <= g * GR:
            lst.append(nxt)
            nxt += 1
        sched.append(lst)
    rest = list(range(nxt, NWD))

    def kernel(q_hbm, k_hbm, v_hbm, o_hbm, qb, kb, vb, ob, sem_in, sem_out):
        def issue_read(g, slot):
            base = g * GR
            n = 0
            for u in range(GR // _RR):
                st = pl.multiple_of(base + u * _RR, _RR)
                for src, dst, off in ((q_hbm, qb, 0), (k_hbm, kb, _PAD), (v_hbm, vb, _PAD)):
                    pltpu.make_async_copy(
                        src.at[pl.ds(st, _RR)],
                        dst.at[pl.ds(pl.multiple_of(st + off, 16), _RR)],
                        sem_in.at[slot],
                    ).start(priority=n % 2)
                    n += 1

        def wait_read(slot):
            tot = qb.at[pl.ds(0, 3 * GR)]
            pltpu.make_async_copy(tot, tot, sem_in.at[slot]).wait()

        def issue_write(j):
            g, cc = divmod(j, nwc)
            sl = (pl.ds(g * _WNH, _WNH), pl.ds(cc * _WR, _WR))
            pltpu.make_async_copy(ob.at[sl], o_hbm.at[sl], sem_out).start()

        for g in range(L):
            issue_read(g, g)
        kb[pl.ds(0, _PAD), :] = jnp.zeros((_PAD, D), kb.dtype)
        vb[pl.ds(0, _PAD), :] = jnp.zeros((_PAD, D), vb.dtype)

        i = lax.broadcasted_iota(jnp.int32, (_TQ, _TK), 0)
        j = lax.broadcasted_iota(jnp.int32, (_TQ, _TK), 1)
        rel = i + _PAD - j
        valid = (rel >= 0) & (rel < _W)
        bias = jnp.where(valid, 0.0, -jnp.inf).astype(jnp.float32)
        bias_first = jnp.where(valid & (j >= _PAD), 0.0, -jnp.inf).astype(jnp.float32)

        def block(sq, og, orow, b):
            qq = qb[pl.ds(sq, _TQ), :]
            kk = kb[pl.ds(sq, _TK), :]
            vv = vb[pl.ds(sq, _TK), :]
            s = lax.dot_general(qq, kk, (((1,), (1,)), ((), ())),
                                preferred_element_type=jnp.float32)
            s = s + b
            m = jnp.max(s, axis=-1, keepdims=True)
            p = jnp.exp2((s - m) * c)
            l = jnp.sum(p, axis=-1, keepdims=True)
            o = jnp.dot(p.astype(vv.dtype), vv, preferred_element_type=jnp.float32)
            r = pl.reciprocal(l, approx=True)
            r = r * (2.0 - l * r)
            ob[og, pl.ds(orow, _TQ), :] = (o * r).astype(ob.dtype)

        def compute_group(g):
            base = g * GR
            og = base // WS
            orow0 = base % WS
            for u in range(GR // _TQ):
                block(pl.multiple_of(base + u * _TQ, _TQ), og,
                      pl.multiple_of(orow0 + u * _TQ, _TQ),
                      bias_first if u == 0 else bias)

        def body(g, carry):
            slot = g % L
            wait_read(slot)
            issue_read(g + L, slot)
            compute_group(g)
            return carry

        lax.fori_loop(0, NG - L, body, 0)
        for idx, g in enumerate(range(NG - L, NG)):
            wait_read(g % L)
            for jw in sched[idx]:
                issue_write(jw)
            compute_group(g)
        for jw in rest:
            issue_write(jw)
        pltpu.make_async_copy(ob, o_hbm, sem_out).wait()

    q2, k2, v2 = (x.reshape(N, D) for x in (q, k, v))
    o = pl.pallas_call(
        kernel,
        in_specs=[pl.BlockSpec(memory_space=pl.ANY)] * 3,
        out_specs=pl.BlockSpec(memory_space=pl.ANY),
        out_shape=jax.ShapeDtypeStruct((_WG, WS, D), q.dtype),
        scratch_shapes=[
            pltpu.VMEM((N, D), q.dtype),
            pltpu.VMEM((N + _PAD, D), k.dtype),
            pltpu.VMEM((N + _PAD, D), v.dtype),
            pltpu.VMEM((_WG, WS, D), q.dtype),
            pltpu.SemaphoreType.DMA((L,)),
            pltpu.SemaphoreType.DMA(()),
        ],
        compiler_params=pltpu.CompilerParams(vmem_limit_bytes=100 * 1024 * 1024),
    )(q2, k2, v2)
    return o.reshape(B, H, S, D)
```

```python
import math

import jax
import jax.numpy as jnp
from jax import lax
from jax.experimental import pallas as pl
from jax.experimental.pallas import tpu as pltpu

_W = 32
_TQ = 64
_TK = 128
_OFF = _TK - _TQ
_RR = 128
_L = 3
_NB = 5
_DEFER = 1
_WNH = 8
_WR = 128


@jax.jit
def pallas_standalone__sliding_local_fixed_window__prompt_kernel(
    q: jax.Array,
    k: jax.Array,
    v: jax.Array,
):
    B, H, S, D = q.shape
    NG = B * H
    N = NG * S
    L = _L
    HR = S // 2
    nu = HR // _RR
    WG = 2 * _WNH
    assert D == 128 and HR % _RR == 0 and S % _TQ == 0 and S >= _TK
    assert NG % WG == 0 and NG > L + 1 and _NB <= nu and _DEFER < L
    WS = N // WG
    assert WS % _WR == 0
    nwc = WS // _WR
    NWD = (WG // _WNH) * nwc
    c = (D ** -0.5) * math.log2(math.e)

    def w_last_row(j):
        g, cc = divmod(j, nwc)
        return (g * _WNH + _WNH - 1) * WS + (cc + 1) * _WR

    n_early = sum(w_last_row(j) <= (NG - 1 - _DEFER) * S for j in range(NWD))

    def kernel(q_hbm, k_hbm, v_hbm, o_hbm, qb, kb, vb, ob, sem_in, sem_tail, sem_out):
        def issue_read(g):
            last = isinstance(g, int) and g == NG - 1
            for u in range(nu):
                sem = sem_tail if (last and u >= nu - _NB) else sem_in.at[g % L]
                for src, dst in ((q_hbm, qb), (k_hbm, kb), (v_hbm, vb)):
                    for half in range(2):
                        sl = pl.ds(pl.multiple_of(g * S + half * HR + u * _RR, _RR), _RR)
                        pltpu.make_async_copy(src.at[sl], dst.at[sl], sem).start(
                            priority=1 - half)

        def wait_rows(sem, rows):
            tot = qb.at[pl.ds(0, rows)]
            pltpu.make_async_copy(tot, tot, sem).wait()

        def wait_read(g):
            last = isinstance(g, int) and g == NG - 1
            wait_rows(sem_in.at[g % L], 3 * S - (6 * _RR * _NB if last else 0))

        def issue_write(j):
            g, cc = divmod(j, nwc)
            sl = (pl.ds(g * _WNH, _WNH), pl.ds(cc * _WR, _WR))
            pltpu.make_async_copy(ob.at[sl], o_hbm.at[sl], sem_out).start()

        for g in range(L):
            issue_read(g)

        row = lax.broadcasted_iota(jnp.int32, (_TQ, _TK), 0)
        col = lax.broadcasted_iota(jnp.int32, (_TQ, _TK), 1)

        def band(off):
            rel = row + off - col
            return (rel >= 0) & (rel < _W)

        mask_mid = band(_OFF)
        mask_first = band(0)

        def block(sq, sk, og, orow, mask):
            qq = qb[pl.ds(sq, _TQ), :]
            kk = kb[pl.ds(sk, _TK), :]
            vv = vb[pl.ds(sk, _TK), :]
            s = lax.dot_general(qq, kk, (((1,), (1,)), ((), ())),
                                preferred_element_type=jnp.float32)
            s = jnp.where(mask, s, -jnp.inf)
            m = jnp.max(s, axis=-1, keepdims=True)
            p = jnp.exp2((s - m) * c)
            l = jnp.sum(p, axis=-1, keepdims=True)
            o = jnp.dot(p.astype(vv.dtype), vv, preferred_element_type=jnp.float32)
            r = pl.reciprocal(l, approx=True)
            r = r * (2.0 - l * r)
            ob[og, pl.ds(orow, _TQ), :] = (o * r).astype(ob.dtype)

        def compute_head(g):
            base = g * S
            og = base // WS
            orow0 = base % WS
            for u in range(S // _TQ):
                sq = pl.multiple_of(base + u * _TQ, _TQ)
                sk = sq if u == 0 else pl.multiple_of(base + u * _TQ - _OFF, _OFF)
                block(sq, sk, og, pl.multiple_of(orow0 + u * _TQ, _TQ),
                      mask_first if u == 0 else mask_mid)

        def loop(lo, hi, fn):
            if hi - lo == 1:
                fn(lo)
            elif hi > lo:
                lax.fori_loop(lo, hi, lambda g, carry: (fn(g), carry)[1], 0)

        def steady(g):
            wait_read(g)
            issue_read(g + L)
            compute_head(g)

        def drain(g):
            wait_read(g)
            compute_head(g)

        loop(0, NG - L - 1, steady)
        steady(NG - L - 1)
        first_deferred = NG - 1 - _DEFER
        loop(NG - L, first_deferred, drain)
        for g in range(first_deferred, NG):
            wait_read(g)
        for j in range(n_early):
            issue_write(j)
        wait_rows(sem_tail, 6 * _RR * _NB)
        loop(first_deferred, NG, compute_head)
        for j in range(n_early, NWD):
            issue_write(j)
        pltpu.make_async_copy(ob, o_hbm, sem_out).wait()

    q2, k2, v2 = (x.reshape(N, D) for x in (q, k, v))
    o = pl.pallas_call(
        kernel,
        in_specs=[pl.BlockSpec(memory_space=pl.ANY)] * 3,
        out_specs=pl.BlockSpec(memory_space=pl.ANY),
        out_shape=jax.ShapeDtypeStruct((WG, WS, D), q.dtype),
        scratch_shapes=[
            pltpu.VMEM((N, D), q.dtype),
            pltpu.VMEM((N, D), k.dtype),
            pltpu.VMEM((N, D), v.dtype),
            pltpu.VMEM((WG, WS, D), q.dtype),
            pltpu.SemaphoreType.DMA((L,)),
            pltpu.SemaphoreType.DMA(()),
            pltpu.SemaphoreType.DMA(()),
        ],
        compiler_params=pltpu.CompilerParams(
            vmem_limit_bytes=100 * 1024 * 1024,
            disable_bounds_checks=True,
        ),
    )(q2, k2, v2)
    return o.reshape(B, H, S, D)
```
